```python
import os as _os
_os.environ.setdefault("JAX_PLATFORMS", "cpu")
import jax
import jax.numpy as jnp

def _softmax(x, axis=-1):
    return jax.nn.softmax(x, axis=axis)
def _gelu(x):
    return jax.nn.gelu(x, approximate=True)
def _silu(x):
    return jax.nn.silu(x)
def _sigmoid(x):
    return jax.nn.sigmoid(x)
def _layernorm(x, axis=-1, eps=1e-5):
    m = jnp.mean(x, axis=axis, keepdims=True)
    v = jnp.var(x, axis=axis, keepdims=True)
    return (x - m) / jnp.sqrt(v + eps)
def _scatter_add(tgt, idx, src, axis=0):
    return tgt.at[idx].add(src)
def _segment_sum(src, seg, n):
    return jax.ops.segment_sum(src, seg, n)
class _Rng:
    def __init__(self, key):
        self._k = key
    def _next(self):
        self._k, sub = jax.random.split(self._k)
        return sub
    def normal(self, shape):
        return jax.random.normal(self._next(), shape, dtype=jnp.bfloat16)
    def randint(self, lo, hi, shape):
        return jax.random.randint(self._next(), shape, lo, hi, dtype=jnp.int32)
    def uniform(self, shape, lo=0.0, hi=1.0):
        return jax.random.uniform(self._next(), shape, jnp.bfloat16, lo, hi)
    def permutation(self, n):
        return jax.random.permutation(self._next(), n)


kernel_name = 'concat_heads__sliding_block_cached__sliding_block_cached__decode'

def setup_inputs():
    _rng = _Rng(jax.random.key(int.from_bytes(__import__("os").urandom(4), "little")))
    _w = (lambda a: (lambda t: t.astype(jnp.bfloat16) if jnp.issubdtype(t.dtype, jnp.floating) else t)(jnp.asarray(a)))
    def _A_setup():
        B, Sq, D = 4, 1, 576
        Hq, Hkv, Sk, Dh = 32, 16, 8192, 128
        assert Hq % Hkv == 0, (Hq, Hkv)
        return {
            "x": _w((lambda *s: _rng.normal(s) * 0.8)(B, Sq, D)),
            "k_cache": _w((lambda *s: _rng.normal(s) * 0.8)(B, Hkv, Sk, Dh)),
            "v_cache": _w((lambda *s: _rng.normal(s) * 0.05)(B, Hkv, Sk, Dh)),
            "wq": _w((lambda *s: _rng.normal(s) * 0.8)(D, Hq * Dh) * (D ** -0.5)),
            "wo": _w((lambda *s: _rng.normal(s) * 0.05)(Hq * Dh, D) * ((Hq * Dh) ** -0.5)),
        }
    _A_in = _A_setup()

    def _B_setup():
        B, Sq, D = 4, 1, 576
        Hq, Hkv, Sk, Dh = 32, 16, 8192, 128
        assert Hq % Hkv == 0, (Hq, Hkv)
        return {
            "x": _w((lambda *s: _rng.normal(s) * 0.8)(B, Sq, D)),
            "k_cache": _w((lambda *s: _rng.normal(s) * 0.8)(B, Hkv, Sk, Dh)),
            "v_cache": _w((lambda *s: _rng.normal(s) * 0.05)(B, Hkv, Sk, Dh)),
            "wq": _w((lambda *s: _rng.normal(s) * 0.8)(D, Hq * Dh) * (D ** -0.5)),
            "wo": _w((lambda *s: _rng.normal(s) * 0.05)(Hq * Dh, D) * ((Hq * Dh) ** -0.5)),
        }
    _B_in = _B_setup()

    return {
        "A_x": _A_in["x"],
        "A_k_cache": _A_in["k_cache"],
        "A_v_cache": _A_in["v_cache"],
        "A_wq": _A_in["wq"],
        "A_wo": _A_in["wo"],
        "B_x": _B_in["x"],
        "B_k_cache": _B_in["k_cache"],
        "B_v_cache": _B_in["v_cache"],
        "B_wq": _B_in["wq"],
        "B_wo": _B_in["wo"],
    }

def reference(A_x, A_k_cache, A_v_cache, A_wq, A_wo, B_x, B_k_cache, B_v_cache, B_wq, B_wo):
    def _A_ref(x, k_cache, v_cache, wq, wo):
        B, Sq, D = x.shape
        Hq, Dh = 32, 128
        Hkv, Sk = k_cache.shape[1], k_cache.shape[2]
        W = min(4096, max(256, Sk // 4))
        rep = Hq // Hkv
        q = (lambda x, *d: x.transpose(*d))((x @ wq).reshape(B, Sq, Hq, Dh), 0, 2, 1, 3)
        k = jnp.repeat(k_cache[:, :, Sk - W:, :], rep, axis=1)
        v = jnp.repeat(v_cache[:, :, Sk - W:, :], rep, axis=1)
        scores = jnp.einsum("bhqd,bhkd->bhqk", q, k) * (Dh ** -0.5)
        p = _softmax(scores, axis=-1)
        o = jnp.einsum("bhqk,bhkd->bhqd", p, v)
        return (lambda x, *d: x.transpose(*d))(o, 0, 2, 1, 3).reshape(B, Sq, Hq * Dh) @ wo

    def _B_ref(x, k_cache, v_cache, wq, wo):
        B, Sq, D = x.shape
        Hq, Dh = 32, 128
        Hkv, Sk = k_cache.shape[1], k_cache.shape[2]
        W = min(4096, max(256, Sk // 4))
        rep = Hq // Hkv
        q = (lambda x, *d: x.transpose(*d))((x @ wq).reshape(B, Sq, Hq, Dh), 0, 2, 1, 3)
        k = jnp.repeat(k_cache[:, :, Sk - W:, :], rep, axis=1)
        v = jnp.repeat(v_cache[:, :, Sk - W:, :], rep, axis=1)
        scores = jnp.einsum("bhqd,bhkd->bhqk", q, k) * (Dh ** -0.5)
        p = _softmax(scores, axis=-1)
        o = jnp.einsum("bhqk,bhkd->bhqd", p, v)
        return (lambda x, *d: x.transpose(*d))(o, 0, 2, 1, 3).reshape(B, Sq, Hq * Dh) @ wo

    a = _A_ref(A_x, A_k_cache, A_v_cache, A_wq, A_wo)
    b = _B_ref(B_x, B_k_cache, B_v_cache, B_wq, B_wo)
    return jnp.concatenate([a, b], axis=-1)
```

```python
import jax
import jax.numpy as jnp
import jax.experimental.pallas as pl
import jax.experimental.pallas.tpu as pltpu

_NT = (((1,), (1,)), ((), ()))
_NN = (((1,), (0,)), ((), ()))
_HQ = 32
_DH = 128
_SLOTS = 4


def _dot(a, b, dims):
    return jax.lax.dot_general(a, b, dims, preferred_element_type=jnp.float32)


@jax.jit
def pallas_concat_heads__sliding_block_cached__sliding_block_cached__decode_kernel(
    A_x, A_k_cache, A_v_cache, A_wq, A_wo, B_x, B_k_cache, B_v_cache, B_wq, B_wo,
):
    nb, sq, d = A_x.shape
    hkv, sk = A_k_cache.shape[1], A_k_cache.shape[2]
    w = min(4096, max(256, sk // 4))
    s0 = sk - w
    scale = _DH ** -0.5
    nu = 2 * hkv

    def kernel(ax, ak, av, awq, awo, bx, bk, bv, bwq, bwo, o_ref,
               xbuf, kbuf, vbuf, qbuf, obuf, acc, xsem, sem):
        def copies(k, v, wq, wo, h, slot):
            cols = pl.ds(pl.multiple_of(h * 2 * _DH, 2 * _DH), 2 * _DH)
            cs = [pltpu.make_async_copy(wq.at[:, cols], qbuf.at[slot], sem.at[slot, 0])]
            cs += [pltpu.make_async_copy(k.at[b, h, pl.ds(s0, w)], kbuf.at[slot, b], sem.at[slot, 1 + b]) for b in range(nb)]
            cs += [pltpu.make_async_copy(v.at[b, h, pl.ds(s0, w)], vbuf.at[slot, b], sem.at[slot, 5 + b]) for b in range(nb)]
            cs += [pltpu.make_async_copy(wo.at[:, cols], obuf.at[slot], sem.at[slot, 9])]
            return cs

        def start(refs, h, slot):
            for i, c in enumerate(copies(*refs, h, slot)):
                c.start(priority=i % 2)

        xc = [pltpu.make_async_copy(x, xbuf.at[i], xsem) for i, x in enumerate((ax, bx))]
        for c in xc:
            c.start()
        for u in range(_SLOTS - 1):
            start((ak, av, awq, awo), u, u)
        for c in xc:
            c.wait()
        acc[...] = jnp.zeros(acc.shape, acc.dtype)
        row = jax.lax.broadcasted_iota(jnp.int32, (8, 1), 0)

        def body(u, _):
            slot = u % _SLOTS
            nxt = u + _SLOTS - 1
            nslot = nxt % _SLOTS
            pl.when(nxt < hkv)(lambda: start((ak, av, awq, awo), nxt, nslot))
            pl.when((nxt >= hkv) & (nxt < nu))(lambda: start((bk, bv, bwq, bwo), nxt - hkv, nslot))
            cs = copies(ak, av, awq, awo, 0, slot)
            side = u // hkv
            x = xbuf[side].astype(jnp.float32)
            x8 = jnp.concatenate([x, x], axis=0).astype(jnp.bfloat16)
            cs[0].wait()
            q8 = _dot(x8, qbuf[slot], _NN)
            q = jnp.where(row < nb, q8[:, :_DH], q8[:, _DH:]).astype(jnp.bfloat16)
            s = None
            for b in range(nb):
                cs[1 + b].wait()
                sb = _dot(q, kbuf[slot, b], _NT)
                s = sb if s is None else jnp.where(row % nb == b, sb, s)
            s = s * scale
            e = jnp.exp(s - jnp.max(s, axis=-1, keepdims=True))
            l = jnp.sum(e, axis=-1, keepdims=True)
            p = e.astype(jnp.bfloat16)
            o = None
            for b in range(nb):
                cs[5 + b].wait()
                ob = _dot(p, vbuf[slot, b], _NN)
                o = ob if o is None else jnp.where(row % nb == b, ob, o)
            o = o / l
            o2 = jnp.concatenate([o, pltpu.roll(o, nb, 0)], axis=1).astype(jnp.bfloat16)
            cs[9].wait()
            acc[side] += _dot(o2, obuf[slot], _NT)

        jax.lax.fori_loop(0, nu, body, None)
        o_ref[...] = jnp.concatenate([acc[0, :nb], acc[1, :nb]], axis=1).astype(o_ref.dtype)

    hbm = pl.BlockSpec(memory_space=pltpu.HBM)
    out = pl.pallas_call(
        kernel,
        out_shape=jax.ShapeDtypeStruct((nb, 2 * d), A_x.dtype),
        in_specs=[hbm] * 10,
        out_specs=pl.BlockSpec(memory_space=pltpu.VMEM),
        scratch_shapes=[
            pltpu.VMEM((2, nb, d), jnp.bfloat16),
            pltpu.VMEM((_SLOTS, nb, w, _DH), jnp.bfloat16),
            pltpu.VMEM((_SLOTS, nb, w, _DH), jnp.bfloat16),
            pltpu.VMEM((_SLOTS, d, 2 * _DH), jnp.bfloat16),
            pltpu.VMEM((_SLOTS, d, 2 * _DH), jnp.bfloat16),
            pltpu.VMEM((2, 8, d), jnp.float32),
            pltpu.SemaphoreType.DMA(()),
            pltpu.SemaphoreType.DMA((_SLOTS, 10)),
        ],
        compiler_params=pltpu.CompilerParams(vmem_limit_bytes=64 * 2**20),
    )(
        A_x.reshape(nb, d), A_k_cache, A_v_cache, A_wq, A_wo.T,
        B_x.reshape(nb, d), B_k_cache, B_v_cache, B_wq, B_wo.T,
    )
    return out.reshape(nb, sq, 2 * d)
```

```python
import functools
import jax
import jax.numpy as jnp
import jax.experimental.pallas as pl
import jax.experimental.pallas.tpu as pltpu

_NT = (((1,), (1,)), ((), ()))
_NN = (((1,), (0,)), ((), ()))
_DH = 128

def _dot(a, b, dims):
    return jax.lax.dot_general(a, b, dims, preferred_element_type=jnp.float32)

def build(RC=256, RR=32, NPC=4, HG=8, CC=512, NOCHK=False, EARLY=False, flags=None):
  def fn(A_x, A_k_cache, A_v_cache, A_wq, A_wo, B_x, B_k_cache, B_v_cache, B_wq, B_wo):
    nb, sq, d = A_x.shape
    hkv, sk = A_k_cache.shape[1], A_k_cache.shape[2]
    hd = A_wq.shape[1]
    rep = hd // _DH // hkv
    w = min(4096, max(256, sk // 4))
    s0 = sk - w
    scale = _DH ** -0.5
    nc = w // RC
    ng = hkv // HG
    ups = ng * nb
    nu = 2 * ups
    nq = HG * rep
    WG = 4; WR = d // WG; WC = 512
    nwc = hd // WC
    assert nwc % nc == 0
    wps = nwc // nc
    hpc = WC // _DH

    def kernel(ax, ak, av, awq, awo, bx, bk, bv, bwq, bwo, o_ref,
               xbuf, kbuf, vbuf, wqbuf, wobuf, qo, sbuf, pbuf, wsem, ksem, vsem):
        def issue_kv(src, buf, sem, u, c):
            b = u % nb; h0 = (u // nb) * HG
            for r in range(RC // RR):
                for g in range(HG // NPC):
                    pltpu.make_async_copy(
                        src.at[b, pl.ds(h0 + g * NPC, NPC), pl.ds(s0 + c * RC + r * RR, RR)],
                        buf.at[c, pl.ds(g * NPC, NPC), pl.ds(r * RR, RR)], sem.at[c]).start(priority=g % 2)

        def issue_wo(src, side, sem, c):
            j = 0
            for r in range(WR // 8):
                for i in range(wps):
                    cc = c * wps + i
                    pltpu.make_async_copy(
                        src.at[:, pl.ds(r * 8, 8), pl.ds(pl.multiple_of(cc * WC, WC), WC)],
                        wobuf.at[side, cc, :, pl.ds(r * 8, 8)], sem.at[c]).start(priority=j % 2)
                    j += 1

        def issue_next(a_src, b_src, wo_src, side, buf, sem, u, c):
            pl.when(u < ups)(lambda: issue_kv(a_src, buf, sem, u, c))
            pl.when((u >= ups) & (u < nu))(lambda: issue_kv(b_src, buf, sem, u - ups, c))
            pl.when(u == nu)(lambda: issue_wo(wo_src, side, sem, c))

        @pl.loop(0, WR // 8)
        def _(r):
            r8 = pl.multiple_of(r * 8, 8)
            for cc in range(nwc):
                for side, src in enumerate((awq, bwq)):
                    pltpu.make_async_copy(src.at[:, pl.ds(r8, 8), pl.ds(cc * WC, WC)],
                                          wqbuf.at[side, cc, :, pl.ds(r8, 8)], wsem).start(priority=side)
        xc = [pltpu.make_async_copy(x, xbuf.at[i], wsem) for i, x in enumerate((ax, bx))]
        for i, c in enumerate(xc):
            c.start(priority=i)
        pl.loop(0, nc)(lambda c: issue_kv(ak, kbuf, ksem, 0, c))
        pl.loop(0, nc)(lambda c: issue_kv(av, vbuf, vsem, 0, c))
        for c in xc:
            c.wait()
        pltpu.make_async_copy(wqbuf, wqbuf, wsem).wait()

        kvh = jax.lax.broadcasted_iota(jnp.int32, (nq, 1), 0) // rep

        def pick(parts):
            out = parts[0]
            for j in range(1, len(parts)):
                out = jnp.where(kvh == j, parts[j], out)
            return out

        @pl.loop(0, nu)
        def _(u):
            side = u // ups
            b = u % nb
            g = u // nb

            @pl.when(b == 0)
            def _():
                x = xbuf[side].astype(jnp.float32)
                x8 = jnp.concatenate([x, jnp.zeros((8 - nb, d), jnp.float32)], axis=0).astype(jnp.bfloat16)
                @pl.loop(0, nq // hpc)
                def _(i):
                    cc = (g % ng) * (nq // hpc) + i
                    q8 = _dot(x8, wqbuf[side, cc].reshape(d, WC), _NN)
                    base = (side * nwc + cc) * hpc * 8
                    for t in range(hpc):
                        qo[pl.ds(pl.multiple_of(base + t * 8, 8), 8), :] = q8[:, t * _DH:(t + 1) * _DH]

            rows = pl.ds(g * nq * 8 + b, nq, stride=8)
            q = qo[rows, :].astype(jnp.bfloat16)

            @pl.loop(0, nc)
            def _(c):
                pltpu.make_async_copy(kbuf.at[c], kbuf.at[c], ksem.at[c]).wait()
                s = _dot(q, kbuf[c].reshape(HG * RC, _DH), _NT)
                sbuf[c] = pick([s[:, j * RC:(j + 1) * RC] for j in range(HG)]) * scale
                issue_next(ak, bk, awo, 0, kbuf, ksem, u + 1, c)

            m = sbuf[0]
            for c in range(1, nc):
                m = jnp.maximum(m, sbuf[c])
            m = jnp.max(m, axis=-1, keepdims=True)
            l = None
            for c in range(nc):
                e = jnp.exp(sbuf[c] - m)
                l = e if l is None else l + e
                pbuf[c] = e.astype(jnp.bfloat16)
            l = jnp.sum(l, axis=-1, keepdims=True)

            def vstep(c, o):
                pltpu.make_async_copy(vbuf.at[c], vbuf.at[c], vsem.at[c]).wait()
                p = pbuf[c]
                o = o + pick([_dot(p, vbuf[c, j], _NN) for j in range(HG)])
                issue_next(av, bv, bwo, 1, vbuf, vsem, u + 1, c)
                return o
            o = jax.lax.fori_loop(0, nc, vstep, jnp.zeros((nq, _DH), jnp.float32))
            qo[rows, :] = o / l

        outs = []
        for side, sem in enumerate((ksem, vsem)):
            def ostep(c, acc, side=side, sem=sem):
                dst = wobuf.at[side, pl.ds(c * wps, wps)]
                pltpu.make_async_copy(dst, dst, sem.at[c]).wait()
                for i in range(wps):
                    cc = c * wps + i
                    base = (side * nwc + cc) * hpc * 8
                    o8 = jnp.concatenate(
                        [qo[pl.ds(pl.multiple_of(base + t * 8, 8), 8), :] for t in range(hpc)], axis=1)
                    acc = acc + _dot(o8.astype(jnp.bfloat16), wobuf[side, cc].reshape(d, WC), _NT)
                return acc
            outs.append(jax.lax.fori_loop(0, nc, ostep, jnp.zeros((8, d), jnp.float32))[:nb])
        o_ref[...] = jnp.concatenate(outs, axis=1).astype(o_ref.dtype)

    hbm = pl.BlockSpec(memory_space=pltpu.HBM)
    wv = lambda a: a.reshape(WG, WR, hd)
    out = pl.pallas_call(
        kernel,
        out_shape=jax.ShapeDtypeStruct((nb, 2 * d), A_x.dtype),
        in_specs=[hbm] * 10,
        out_specs=pl.BlockSpec(memory_space=pltpu.VMEM),
        scratch_shapes=[
            pltpu.VMEM((2, nb, d), jnp.bfloat16),
            pltpu.VMEM((nc, HG, RC, _DH), jnp.bfloat16),
            pltpu.VMEM((nc, HG, RC, _DH), jnp.bfloat16),
            pltpu.VMEM((2, nwc, WG, WR, WC), jnp.bfloat16),
            pltpu.VMEM((2, nwc, WG, WR, WC), jnp.bfloat16),
            pltpu.VMEM((2 * hd // _DH * 8, _DH), jnp.float32),
            pltpu.VMEM((nc, nq, RC), jnp.float32),
            pltpu.VMEM((nc, nq, RC), jnp.bfloat16),
            pltpu.SemaphoreType.DMA(()),
            pltpu.SemaphoreType.DMA((nc,)),
            pltpu.SemaphoreType.DMA((nc,)),
        ],
        compiler_params=pltpu.CompilerParams(vmem_limit_bytes=64 * 2**20, disable_bounds_checks=NOCHK, flags=flags),
    )(
        A_x.reshape(nb, d), A_k_cache, A_v_cache, wv(A_wq), wv(A_wo.T),
        B_x.reshape(nb, d), B_k_cache, B_v_cache, wv(B_wq), wv(B_wo.T),
    )
    return out.reshape(nb, sq, 2 * d)
  return fn

pallas_concat_heads__sliding_block_cached__sliding_block_cached__decode_kernel = jax.jit(build(RC=512))
```

```python
import functools

import jax
import jax.numpy as jnp
import jax.experimental.pallas as pl
import jax.experimental.pallas.tpu as pltpu

_DH = 128
_SUB = 8
_LANE = 128
_ROWS = 256
_RING = 4
_KV_COPY = (2, 64)
_GROUP = 8
_W_BANDS = 4
_W_COLS = 1024
_T_COLS = 512
_T_ROWS = 32

_NN = (((1,), (0,)), ((), ()))
_NT = (((1,), (1,)), ((), ()))


def _dot(a, b, dims):
    return jax.lax.dot_general(a, b, dims, preferred_element_type=jnp.float32)


def _wait_all(dst, sem):
    pltpu.make_async_copy(dst, dst, sem).wait()


def _kernel(
    ax, ak, av, awq, awo, bx, bk, bv, bwq, bwo, o_ref,
    xbuf, ring, wbuf, tbuf, qo, sbuf, pbuf, lbuf, oacc, aacc,
    xsem, wsem, rsem, tsem, *, window,
):
    nb, d = ax.shape
    hkv, sk = ak.shape[1], ak.shape[2]
    hq = awq.shape[-1] // _DH
    rep = hq // hkv
    start = sk - window
    nc = window // _ROWS
    ns = 2 * nb * 2 * nc
    ng, nq = hkv // _GROUP, _GROUP * rep
    nw, nt = wbuf.shape[1], tbuf.shape[0]
    pad = tbuf.shape[1] - d

    def start_stage(src, n):
        b, c, slot = (n // (2 * nc)) % nb, n % nc, n % _RING
        nh, nr = _KV_COPY
        for r in range(_ROWS // nr):
            for g in range(hkv // nh):
                pltpu.make_async_copy(
                    src.at[b, pl.ds(g * nh, nh), pl.ds(start + c * _ROWS + r * nr, nr)],
                    ring.at[slot, pl.ds(g * nh, nh), pl.ds(r * nr, nr)],
                    rsem.at[slot],
                ).start(priority=g % 2)

    def start_tail(t):
        cols = pl.ds(pl.multiple_of(t * _T_COLS, _T_COLS), _T_COLS)
        for r in range(d // _T_ROWS):
            pltpu.make_async_copy(
                bwo.at[pl.ds(r * _T_ROWS, _T_ROWS), cols],
                tbuf.at[t, pl.ds(pad + r * _T_ROWS, _T_ROWS)],
                tsem.at[t],
            ).start(priority=r % 2)

    def start_next(n):
        which = (n // (ns // 2)) * 2 + (n // nc) % 2
        for i, src in enumerate((ak, av, bk, bv)):
            pl.when(which == i)(functools.partial(start_stage, src, n))

        @pl.when(n >= ns)
        def _():
            per = nt // _RING
            pl.loop(0, per)(lambda i: start_tail((n - ns) * per + i))

    def head_rows(h):
        return pl.ds(pl.multiple_of(h * _SUB, _SUB), _SUB)

    def project_q(side, cc):
        x = xbuf[side].astype(jnp.float32)
        x = jnp.concatenate([x, jnp.zeros((_SUB - nb, d), jnp.float32)], axis=0)
        q = _dot(x.astype(wbuf.dtype), wbuf[side, cc].reshape(d, _W_COLS), _NN)
        for t in range(_W_COLS // _DH):
            h = side * hq + cc * (_W_COLS // _DH) + t
            qo[head_rows(h), :] = q[:, t * _DH:(t + 1) * _DH]

    def head_outputs(h0, n):
        o = jnp.concatenate([qo[head_rows(h0 + t), :] for t in range(n)], axis=1)
        return o.astype(wbuf.dtype)

    @pl.loop(0, wbuf.shape[3] // _SUB)
    def _(r):
        rows = pl.ds(pl.multiple_of(r * _SUB, _SUB), _SUB)
        j = 0
        for cc in range(nw):
            for g in range(0, _W_BANDS, 2):
                for i, src in enumerate((awq, bwq, awo)):
                    pltpu.make_async_copy(
                        src.at[pl.ds(g, 2), rows, pl.ds(cc * _W_COLS, _W_COLS)],
                        wbuf.at[i, cc, pl.ds(g, 2), rows],
                        wsem,
                    ).start(priority=j % 2)
                    j += 1

    x_copies = [
        pltpu.make_async_copy(x, xbuf.at[i], xsem.at[i]) for i, x in enumerate((ax, bx))
    ]
    for i, copy in enumerate(x_copies):
        copy.start(priority=i)
    pl.loop(0, _RING)(functools.partial(start_stage, ak))

    aacc[...] = jnp.zeros(aacc.shape, aacc.dtype)
    tbuf[:, :pad, :] = jnp.zeros((nt, pad, _T_COLS), tbuf.dtype)
    for copy in x_copies:
        copy.wait()
    _wait_all(wbuf, wsem)
    pl.loop(0, nw)(functools.partial(project_q, 0))

    kv_head = jax.lax.broadcasted_iota(jnp.int32, (nq, 1), 0) // rep

    def pick(parts):
        out = parts[0]
        for j in range(1, len(parts)):
            out = jnp.where(kv_head == j, parts[j], out)
        return out

    @pl.loop(0, ns)
    def _(s):
        slot, c, unit = s % _RING, s % nc, s // (2 * nc)
        is_v = (s // nc) % 2
        rows = [
            pl.ds(((unit // nb) * hq + g * nq) * _SUB + unit % nb, nq, stride=_SUB)
            for g in range(ng)
        ]
        _wait_all(ring.at[slot], rsem.at[slot])

        @pl.when(is_v == 0)
        def _():
            for g in range(ng):
                q = qo[rows[g], :].astype(ring.dtype)
                k = ring[slot, pl.ds(g * _GROUP, _GROUP)].reshape(_GROUP * _ROWS, _DH)
                sc = _dot(q, k, _NT)
                sc = pick([sc[:, j * _ROWS:(j + 1) * _ROWS] for j in range(_GROUP)])
                sbuf[g, c] = sc * (_DH ** -0.5)

            @pl.when(c == nc - 1)
            def _():
                for g in range(ng):
                    m = functools.reduce(jnp.maximum, [sbuf[g, i] for i in range(nc)])
                    m = jnp.max(m, axis=-1, keepdims=True)
                    total = None
                    for i in range(nc):
                        e = jnp.exp(sbuf[g, i] - m)
                        total = e if total is None else total + e
                        pbuf[g, i] = e.astype(pbuf.dtype)
                    total = jnp.sum(total, axis=-1, keepdims=True)
                    lbuf[g] = jnp.broadcast_to(total, (nq, _DH))
                    oacc[g] = jnp.zeros((nq, _DH), jnp.float32)

        @pl.when(is_v == 1)
        def _():
            for g in range(ng):
                p = pbuf[g, c]
                oacc[g] += pick(
                    [_dot(p, ring[slot, g * _GROUP + j], _NN) for j in range(_GROUP)]
                )

            @pl.when(c == nc - 1)
            def _():
                for g in range(ng):
                    qo[rows[g], :] = oacc[g] / lbuf[g]

        start_next(s + _RING)

        pl.when((s >= nc) & (s < nc + nw))(lambda: project_q(1, s - nc))
        cc = s - (ns // 2 + nc)

        @pl.when((cc >= 0) & (cc < nw))
        def _():
            n = _W_COLS // _DH
            wo = wbuf[2, cc].reshape(d, _W_COLS)
            aacc[...] += _dot(head_outputs(cc * n, n), wo, _NT)

    def project_b(t, acc):
        n = _T_COLS // _DH
        o = head_outputs(hq + t * n, n)
        _wait_all(tbuf.at[t, pl.ds(pad, d)], tsem.at[t])
        return acc + _dot(o, tbuf[t], _NT)

    seam = d - pad
    o_ref[:, :seam] = aacc[:nb, :seam].astype(o_ref.dtype)
    a_edge = jnp.concatenate(
        [aacc[:, seam:], jnp.zeros((_SUB, _LANE - pad), jnp.float32)], axis=1
    )
    out_b = jax.lax.fori_loop(0, nt, project_b, jnp.zeros((_SUB, pad + d), jnp.float32))
    lane = jax.lax.broadcasted_iota(jnp.int32, (_SUB, _LANE), 1)
    mixed = jnp.where(lane < pad, a_edge, out_b[:, :_LANE])
    o_ref[:, seam:seam + _LANE] = mixed[:nb].astype(o_ref.dtype)
    o_ref[:, seam + _LANE:] = out_b[:nb, _LANE:].astype(o_ref.dtype)


@jax.jit
def pallas_concat_heads__sliding_block_cached__sliding_block_cached__decode_kernel(
    A_x: jax.Array,
    A_k_cache: jax.Array,
    A_v_cache: jax.Array,
    A_wq: jax.Array,
    A_wo: jax.Array,
    B_x: jax.Array,
    B_k_cache: jax.Array,
    B_v_cache: jax.Array,
    B_wq: jax.Array,
    B_wo: jax.Array,
):
    nb, sq, d = A_x.shape
    hkv, sk = A_k_cache.shape[1], A_k_cache.shape[2]
    hd = A_wq.shape[1]
    dt = A_x.dtype
    window = min(4096, max(256, sk // 4))
    hq = hd // _DH
    nc, ng, nq = window // _ROWS, hkv // _GROUP, _GROUP * (hq // hkv)
    nw, nt, band = hd // _W_COLS, hd // _T_COLS, d // _W_BANDS
    assert sq == 1 and nb < _SUB and d % _LANE and d % _T_ROWS == 0 and band % 16 == 0
    assert window % _ROWS == 0 and max(_RING, nw) <= nc and nt % _RING == 0
    assert hkv % _GROUP == 0 and hd % _W_COLS == 0

    def bands(w):
        return w.reshape(_W_BANDS, band, hd)

    out = pl.pallas_call(
        functools.partial(_kernel, window=window),
        out_shape=jax.ShapeDtypeStruct((nb, 2 * d), dt),
        in_specs=[pl.BlockSpec(memory_space=pltpu.HBM)] * 10,
        out_specs=pl.BlockSpec(memory_space=pltpu.VMEM),
        scratch_shapes=[
            pltpu.VMEM((2, nb, d), dt),
            pltpu.VMEM((_RING, hkv, _ROWS, _DH), dt),
            pltpu.VMEM((3, nw, _W_BANDS, band, _W_COLS), dt),
            pltpu.VMEM((nt, d % _LANE + d, _T_COLS), dt),
            pltpu.VMEM(((2 * hq + 1) * _SUB, _DH), jnp.float32),
            pltpu.VMEM((ng, nc, nq, _ROWS), jnp.float32),
            pltpu.VMEM((ng, nc, nq, _ROWS), dt),
            pltpu.VMEM((ng, nq, _DH), jnp.float32),
            pltpu.VMEM((ng, nq, _DH), jnp.float32),
            pltpu.VMEM((_SUB, d), jnp.float32),
            pltpu.SemaphoreType.DMA((2,)),
            pltpu.SemaphoreType.DMA(()),
            pltpu.SemaphoreType.DMA((_RING,)),
            pltpu.SemaphoreType.DMA((nt,)),
        ],
        compiler_params=pltpu.CompilerParams(vmem_limit_bytes=48 * 2**20),
    )(
        A_x.reshape(nb, d), A_k_cache, A_v_cache, bands(A_wq), bands(A_wo.T),
        B_x.reshape(nb, d), B_k_cache, B_v_cache, bands(B_wq), B_wo.T,
    )
    return out.reshape(nb, sq, 2 * d)
```
